```python
import jax
import jax.numpy as jnp

def _softmax(x, axis=-1):
    return jax.nn.softmax(x, axis=axis)
def _gelu(x):
    return jax.nn.gelu(x, approximate=True)
def _silu(x):
    return jax.nn.silu(x)
def _sigmoid(x):
    return jax.nn.sigmoid(x)
def _layernorm(x, axis=-1, eps=1e-5):
    m = jnp.mean(x, axis=axis, keepdims=True)
    v = jnp.var(x, axis=axis, keepdims=True)
    return (x - m) / jnp.sqrt(v + eps)
def _scatter_add(tgt, idx, src, axis=0):
    return tgt.at[idx].add(src)
def _segment_sum(src, seg, n):
    return jax.ops.segment_sum(src, seg, n)
class _Rng:
    def __init__(self, key):
        self._k = key
    def _next(self):
        self._k, sub = jax.random.split(self._k)
        return sub
    def normal(self, shape):
        return jax.random.normal(self._next(), shape, dtype=jnp.bfloat16)
    def randint(self, lo, hi, shape):
        return jax.random.randint(self._next(), shape, lo, hi, dtype=jnp.int32)
    def uniform(self, shape, lo=0.0, hi=1.0):
        return jax.random.uniform(self._next(), shape, jnp.bfloat16, lo, hi)
    def permutation(self, n):
        return jax.random.permutation(self._next(), n)


kernel_name = 'recurrent_scan__sliding_block_cached__moe_arch_mod__prompt'

def setup_inputs():
    _rng = _Rng(jax.random.key(int.from_bytes(__import__("os").urandom(4), "little")))
    _w = (lambda a: (lambda t: t.astype(jnp.bfloat16) if jnp.issubdtype(t.dtype, jnp.floating) else t)(jnp.asarray(a)))
    def _A_setup():
        B, Sq, D = 1, 2048, 640
        Hq, Hkv, Sk, Dh = 32, 32, 2048, 192
        assert Hq % Hkv == 0, (Hq, Hkv)
        return {
            "x": _w((lambda *s: _rng.normal(s) * 0.05)(B, Sq, D)),
            "k_cache": _w((lambda *s: _rng.normal(s) * 0.05)(B, Hkv, Sk, Dh)),
            "v_cache": _w((lambda *s: _rng.normal(s) * 0.05)(B, Hkv, Sk, Dh)),
            "wq": _w((lambda *s: _rng.normal(s) * 0.05)(D, Hq * Dh) * (D ** -0.5)),
            "wo": _w((lambda *s: _rng.normal(s) * 0.05)(Hq * Dh, D) * ((Hq * Dh) ** -0.5)),
        }
    _A_in = _A_setup()

    def _B_setup():
        B, S, D, F, C = 1, 2048, 640, 1536, 2
        return {
            "x": _w((lambda *s: _rng.normal(s) * 0.05)(B, S, D)),
            "w_r": _w((lambda *s: _rng.normal(s) * 0.05)(D)),
            "w_gate": _w((lambda *s: _rng.normal(s) * 0.05)(D, F)),
            "w_up": _w((lambda *s: _rng.normal(s) * 0.05)(D, F)),
            "w_down": _w((lambda *s: _rng.normal(s) * 0.05)(F, D)),
        }
    _B_in = _B_setup()

    return {
        "A_x": _A_in["x"],
        "A_k_cache": _A_in["k_cache"],
        "A_v_cache": _A_in["v_cache"],
        "A_wq": _A_in["wq"],
        "A_wo": _A_in["wo"],
        "B_x": _B_in["x"],
        "B_w_r": _B_in["w_r"],
        "B_w_gate": _B_in["w_gate"],
        "B_w_up": _B_in["w_up"],
        "B_w_down": _B_in["w_down"],
    }

def reference(A_x, A_k_cache, A_v_cache, A_wq, A_wo, B_x, B_w_r, B_w_gate, B_w_up, B_w_down):
    def _A_ref(x, k_cache, v_cache, wq, wo):
        B, Sq, D = x.shape
        Hq, Dh = 32, 192
        Hkv, Sk = k_cache.shape[1], k_cache.shape[2]
        W = min(4096, max(256, Sk // 4))
        rep = Hq // Hkv
        q = (lambda x, *d: x.transpose(*d))((x @ wq).reshape(B, Sq, Hq, Dh), 0, 2, 1, 3)
        k = jnp.repeat(k_cache[:, :, Sk - W:, :], rep, axis=1)
        v = jnp.repeat(v_cache[:, :, Sk - W:, :], rep, axis=1)
        scores = jnp.einsum("bhqd,bhkd->bhqk", q, k) * (Dh ** -0.5)
        p = _softmax(scores, axis=-1)
        o = jnp.einsum("bhqk,bhkd->bhqd", p, v)
        return (lambda x, *d: x.transpose(*d))(o, 0, 2, 1, 3).reshape(B, Sq, Hq * Dh) @ wo

    def _B_ref(x, w_r, w_gate, w_up, w_down):
        B, S, D = x.shape
        C = 2
        r = x @ w_r
        idx = jnp.argsort(-r, axis=-1)[:, :C]
        idx_e = jnp.repeat(idx.reshape(B, C, 1), D, axis=2)
        x_sel = jnp.take_along_axis(x, idx_e, axis=1)
        g = _silu(x_sel @ w_gate)
        u = x_sel @ w_up
        y = (g * u) @ w_down
        r_sel = _sigmoid(jnp.take_along_axis(r, idx, axis=1))
        y = y * r_sel.reshape(B, C, 1)
        b_off = (jnp.arange(B) * S).reshape(B, 1)
        flat_idx = (idx + b_off).reshape(B * C)
        zero = (x * 0.0).reshape(B * S, D)
        upd = _scatter_add(zero, flat_idx, y.reshape(B * C, D), axis=0)
        return x + upd.reshape(B, S, D)

    x = A_x
    xn = _layernorm(x, axis=-1)
    s = _A_ref(xn, A_k_cache, A_v_cache, A_wq, A_wo)
    g = _silu(_B_ref(xn, B_w_r, B_w_gate, B_w_up, B_w_down))
    return x + s * g
```

```python
import functools

import jax
import jax.numpy as jnp
import numpy as np
from jax import lax
import jax.experimental.pallas as pl
import jax.experimental.pallas.tpu as pltpu

S = 2048
D = 640
H = 32
DH = 192
SK = 2048
W = 512
F = 1536
NP = H // 2
TM = 512

_NT = (((1,), (1,)), ((), ()))
_F32 = jnp.float32
_BF16 = jnp.bfloat16


def _kernel(x_ref, k_ref, v_ref, wq_ref, wo_ref, wr_ref, wg_ref, wu_ref, wd_ref,
            o_ref, xn_ref, acc_ref, kp_ref, vp_ref):
    p = pl.program_id(0)

    @pl.when(p == 0)
    def _():
        x = x_ref[0].astype(_F32)
        m = jnp.mean(x, axis=-1, keepdims=True)
        var = jnp.mean(jnp.square(x - m), axis=-1, keepdims=True)
        m_b = m.astype(_BF16).astype(_F32)
        v_b = var.astype(_BF16).astype(_F32)
        d = (x - m_b).astype(_BF16).astype(_F32)
        den = jnp.sqrt((v_b + 1e-5).astype(_BF16).astype(_F32)).astype(_BF16).astype(_F32)
        xn_ref[...] = (d / den).astype(_BF16)
        acc_ref[...] = jnp.zeros_like(acc_ref)

    z = jnp.zeros((64, W), _BF16)
    kp_ref[0] = jnp.concatenate([k_ref[0, 0], z], axis=0)
    kp_ref[1] = jnp.concatenate([z, k_ref[0, 1]], axis=0)
    vp_ref[0] = jnp.concatenate([v_ref[0, 0], z], axis=0)
    vp_ref[1] = jnp.concatenate([z, v_ref[0, 1]], axis=0)

    qscale = np.float32((DH ** -0.5) * np.log2(np.e))

    def tile(i, _):
        r0 = pl.multiple_of(i * TM, TM)
        xn = xn_ref[pl.ds(r0, TM), :]
        q2 = jnp.dot(xn, wq_ref[...], preferred_element_type=_F32)
        q2 = (q2 * qscale).astype(_BF16)
        s0 = jnp.dot(q2[:, 0:256], kp_ref[0], preferred_element_type=_F32)
        s1 = jnp.dot(q2[:, 128:384], kp_ref[1], preferred_element_type=_F32)
        p0 = jnp.exp2(s0 - jnp.max(s0, axis=-1, keepdims=True))
        p1 = jnp.exp2(s1 - jnp.max(s1, axis=-1, keepdims=True))
        i0 = 1.0 / jnp.sum(p0, axis=-1, keepdims=True)
        i1 = 1.0 / jnp.sum(p1, axis=-1, keepdims=True)
        a = lax.dot_general(p0.astype(_BF16), vp_ref[0], _NT, preferred_element_type=_F32) * i0
        b = lax.dot_general(p1.astype(_BF16), vp_ref[1], _NT, preferred_element_type=_F32) * i1
        o2 = jnp.concatenate([a[:, 0:128], a[:, 128:256] + b[:, 0:128], b[:, 128:256]], axis=1)
        acc_ref[pl.ds(r0, TM), :] += jnp.dot(o2.astype(_BF16), wo_ref[...],
                                              preferred_element_type=_F32)
        return 0

    lax.fori_loop(0, S // TM, tile, 0)

    @pl.when(p == NP - 1)
    def _():
        xnf = xn_ref[...].astype(_F32)
        wr = wr_ref[...].astype(_F32)
        r = jnp.sum(xnf * wr, axis=-1, keepdims=True)
        r = r.astype(_BF16).astype(_F32)
        idx = lax.broadcasted_iota(jnp.int32, (S, 1), 0)
        m0 = jnp.max(r)
        i0 = jnp.min(jnp.where(r == m0, idx, S))
        r2 = jnp.where(idx == i0, -jnp.inf, r)
        m1 = jnp.max(r2)
        i1 = jnp.min(jnp.where(r2 == m1, idx, S))
        sel0 = idx == i0
        sel1 = idx == i1
        x0 = jnp.sum(jnp.where(sel0, xnf, 0.0), axis=0, keepdims=True)
        x1 = jnp.sum(jnp.where(sel1, xnf, 0.0), axis=0, keepdims=True)
        row = lax.broadcasted_iota(jnp.int32, (8, D), 0)
        xs = jnp.where(row == 0, x0, jnp.where(row == 1, x1, 0.0)).astype(_BF16)
        gg = jnp.dot(xs, wg_ref[...], preferred_element_type=_F32).astype(_BF16).astype(_F32)
        uu = jnp.dot(xs, wu_ref[...], preferred_element_type=_F32).astype(_BF16).astype(_F32)
        gg = (gg * jax.nn.sigmoid(gg)).astype(_BF16).astype(_F32)
        hh = (gg * uu).astype(_BF16)
        y = jnp.dot(hh, wd_ref[...], preferred_element_type=_F32).astype(_BF16).astype(_F32)
        rs0 = jax.nn.sigmoid(jnp.full((1, 1), m0, _F32)).astype(_BF16).astype(_F32)
        rs1 = jax.nn.sigmoid(jnp.full((1, 1), m1, _F32)).astype(_BF16).astype(_F32)
        y0 = (y[0:1] * rs0).astype(_BF16).astype(_F32)
        y1 = (y[1:2] * rs1).astype(_BF16).astype(_F32)
        t = jnp.where(sel0, xnf + y0, jnp.where(sel1, xnf + y1, xnf))
        t = t.astype(_BF16).astype(_F32)
        g = (t * jax.nn.sigmoid(t)).astype(_BF16).astype(_F32)
        s = acc_ref[...].astype(_BF16).astype(_F32)
        out = x_ref[0].astype(_F32) + (s * g).astype(_BF16).astype(_F32)
        o_ref[0] = out.astype(o_ref.dtype)


@jax.jit
def pallas_recurrent_scan__sliding_block_cached__moe_arch_mod__prompt_kernel(
    A_x: jax.Array,
    A_k_cache: jax.Array,
    A_v_cache: jax.Array,
    A_wq: jax.Array,
    A_wo: jax.Array,
    B_x: jax.Array,
    B_w_r: jax.Array,
    B_w_gate: jax.Array,
    B_w_up: jax.Array,
    B_w_down: jax.Array,
):
    del B_x
    wblk = SK // W - 1
    full = lambda shape: pl.BlockSpec(shape, lambda p: (0,) * len(shape))
    return pl.pallas_call(
        _kernel,
        grid=(NP,),
        in_specs=[
            full((1, S, D)),
            pl.BlockSpec((1, 2, DH, W), lambda p: (0, p, 0, wblk)),
            pl.BlockSpec((1, 2, DH, W), lambda p: (0, p, 0, wblk)),
            pl.BlockSpec((D, 2 * DH), lambda p: (0, p)),
            pl.BlockSpec((2 * DH, D), lambda p: (p, 0)),
            full((1, D)),
            full((D, F)),
            full((D, F)),
            full((F, D)),
        ],
        out_specs=full((1, S, D)),
        out_shape=jax.ShapeDtypeStruct((1, S, D), A_x.dtype),
        scratch_shapes=[
            pltpu.VMEM((S, D), _BF16),
            pltpu.VMEM((S, D), _F32),
            pltpu.VMEM((2, 256, W), _BF16),
            pltpu.VMEM((2, 256, W), _BF16),
        ],
        compiler_params=pltpu.CompilerParams(
            dimension_semantics=("arbitrary",),
            vmem_limit_bytes=100 * 1024 * 1024,
        ),
    )(A_x, jnp.swapaxes(A_k_cache, 2, 3), jnp.swapaxes(A_v_cache, 2, 3), A_wq, A_wo, B_w_r.reshape(1, D), B_w_gate, B_w_up, B_w_down)
```

```python
import functools

import jax
import jax.numpy as jnp
import numpy as np
from jax import lax
import jax.experimental.pallas as pl
import jax.experimental.pallas.tpu as pltpu

S = 2048
D = 640
H = 32
DH = 192
SK = 2048
W = 512
F = 1536
NP = H // 2
TM = 512
NT_ = S // TM

_NT = (((1,), (1,)), ((), ()))
_F32 = jnp.float32
_BF16 = jnp.bfloat16
_QS = np.float32((DH ** -0.5) * np.log2(np.e))


def _dot(a, b):
    return jnp.dot(a, b, preferred_element_type=_F32)


def _dnt(a, b):
    return lax.dot_general(a, b, _NT, preferred_element_type=_F32)


def _rb(a):
    return a.astype(_BF16).astype(_F32)


def _kernel(x_ref, k_ref, v_ref, wq_ref, wo_ref, wr_ref, wg_hbm, wu_hbm, wd_hbm,
            o_ref, xn_ref, acc_ref, kp_ref, wt_ref, wg_ref, wu_ref, wd_ref, sem):
    p = pl.program_id(0)
    ffn_copies = [
        pltpu.make_async_copy(wg_hbm, wg_ref, sem.at[0]),
        pltpu.make_async_copy(wu_hbm, wu_ref, sem.at[1]),
        pltpu.make_async_copy(wd_hbm, wd_ref, sem.at[2]),
    ]

    def layernorm(r0):
        x = x_ref[0, r0:r0 + TM, :].astype(_F32)
        m = jnp.mean(x, axis=-1, keepdims=True)
        d = x - m
        var = jnp.mean(d * d, axis=-1, keepdims=True)
        den = _rb(jnp.sqrt(_rb(_rb(var) + 1e-5)))
        xn = (_rb(x - _rb(m)) / den).astype(_BF16)
        xn_ref[r0:r0 + TM, :] = xn

    def stage_q(r0):
        q2 = _dot(xn_ref[r0:r0 + TM, :], wq_ref[...])
        return (q2 * _QS).astype(_BF16)

    def stage_s(q2):
        return _dot(q2[:, 0:256], kp_ref[0]), _dot(q2[:, 128:384], kp_ref[1])

    def softmax(s):
        e = jnp.exp2(s - jnp.max(s, axis=-1, keepdims=True))
        return (e * (1.0 / jnp.sum(e, axis=-1, keepdims=True))).astype(_BF16)

    def stage_p(s0, s1):
        a = _dnt(v_ref[0, 0], softmax(s0))
        b = _dnt(v_ref[0, 1], softmax(s1))
        return jnp.concatenate([a, b], axis=0).astype(_BF16)

    def stage_o(o2t):
        return _dot(wt_ref[...], o2t)

    def prep():
        z = jnp.zeros((64, W), _BF16)
        kp_ref[0] = jnp.concatenate([k_ref[0, 0], z], axis=0)
        kp_ref[1] = jnp.concatenate([z, k_ref[0, 1]], axis=0)
        wt_ref[...] = wo_ref[...].T

    def attention(first):
        rs = [u * TM for u in range(NT_)]
        qs = [stage_q(r0) for r0 in rs]
        ss = [stage_s(q) for q in qs]
        os_ = [stage_p(*s) for s in ss]
        return [stage_o(o) for o in os_]

    def router_ffn():
        xnf = xn_ref[...].astype(_F32)
        wr = wr_ref[...].astype(_F32)
        r = _rb(jnp.sum(xnf * wr, axis=-1, keepdims=True))
        idx = lax.broadcasted_iota(jnp.int32, (S, 1), 0)
        m0 = jnp.max(r)
        i0 = jnp.min(jnp.where(r == m0, idx, S))
        r2 = jnp.where(idx == i0, -jnp.inf, r)
        m1 = jnp.max(r2)
        i1 = jnp.min(jnp.where(r2 == m1, idx, S))
        i0 = jnp.minimum(i0, S - 1)
        i1 = jnp.minimum(i1, S - 1)
        row16 = lax.broadcasted_iota(jnp.int32, (16, D), 0)

        def gather(i):
            base = pl.multiple_of((i // 16) * 16, 16)
            blk = xn_ref[pl.ds(base, 16), :].astype(_F32)
            return jnp.sum(jnp.where(row16 == i - base, blk, 0.0), axis=0, keepdims=True)

        x0 = gather(i0)
        x1 = gather(i1)
        xs = jnp.where(row16 == 0, x0, jnp.where(row16 == 1, x1, 0.0)).astype(_BF16)
        gg = _rb(_dot(xs, wg_ref[...]))
        uu = _rb(_dot(xs, wu_ref[...]))
        gg = _rb(gg * jax.nn.sigmoid(gg))
        y = _rb(_dot((gg * uu).astype(_BF16), wd_ref[...]))
        rs0 = _rb(jax.nn.sigmoid(jnp.full((1, 1), m0, _F32)))
        rs1 = _rb(jax.nn.sigmoid(jnp.full((1, 1), m1, _F32)))
        return i0, i1, _rb(y[0:1] * rs0), _rb(y[1:2] * rs1)

    def finish(r0, st, i0, i1, y0, y1):
        xnf = xn_ref[r0:r0 + TM, :].astype(_F32)
        idx = lax.broadcasted_iota(jnp.int32, (TM, 1), 0) + r0
        t = jnp.where(idx == i0, xnf + y0, jnp.where(idx == i1, xnf + y1, xnf))
        t = _rb(t)
        g = _rb(t * jax.nn.sigmoid(t))
        s = _rb(st.T)
        out = x_ref[0, r0:r0 + TM, :].astype(_F32) + _rb(s * g)
        o_ref[0, r0:r0 + TM, :] = out.astype(o_ref.dtype)

    @pl.when(p == 0)
    def _():
        for c in ffn_copies:
            c.start()
        for u in range(NT_):
            layernorm(u * TM)
        acc_ref[...] = jnp.zeros_like(acc_ref)

    prep()
    outs = attention(False)
    for u in range(NT_):
        acc_ref[:, u * TM:(u + 1) * TM] += outs[u]

    @pl.when(p == NP - 1)
    def _():
        for c in ffn_copies:
            c.wait()
        i0, i1, y0, y1 = router_ffn()
        for u in range(NT_):
            finish(u * TM, acc_ref[:, u * TM:(u + 1) * TM], i0, i1, y0, y1)


@jax.jit
def pallas_recurrent_scan__sliding_block_cached__moe_arch_mod__prompt_kernel(
    A_x: jax.Array,
    A_k_cache: jax.Array,
    A_v_cache: jax.Array,
    A_wq: jax.Array,
    A_wo: jax.Array,
    B_x: jax.Array,
    B_w_r: jax.Array,
    B_w_gate: jax.Array,
    B_w_up: jax.Array,
    B_w_down: jax.Array,
):
    del B_x
    wblk = SK // W - 1
    full = lambda shape: pl.BlockSpec(shape, lambda p: (0,) * len(shape))
    hbm = pl.BlockSpec(memory_space=pl.ANY)
    return pl.pallas_call(
        _kernel,
        grid=(NP,),
        in_specs=[
            full((1, S, D)),
            pl.BlockSpec((1, 2, DH, W), lambda p: (0, p, 0, wblk)),
            pl.BlockSpec((1, 2, DH, W), lambda p: (0, p, 0, wblk)),
            pl.BlockSpec((D, 2 * DH), lambda p: (0, p)),
            pl.BlockSpec((2 * DH, D), lambda p: (p, 0)),
            full((1, D)),
            hbm, hbm, hbm,
        ],
        out_specs=full((1, S, D)),
        out_shape=jax.ShapeDtypeStruct((1, S, D), A_x.dtype),
        scratch_shapes=[
            pltpu.VMEM((S, D), _BF16),
            pltpu.VMEM((D, S), _F32),
            pltpu.VMEM((2, 256, W), _BF16),
            pltpu.VMEM((D, 2 * DH), _BF16),
            pltpu.VMEM((D, F), _BF16),
            pltpu.VMEM((D, F), _BF16),
            pltpu.VMEM((F, D), _BF16),
            pltpu.SemaphoreType.DMA((3,)),
        ],
        compiler_params=pltpu.CompilerParams(
            dimension_semantics=("arbitrary",),
            vmem_limit_bytes=100 * 1024 * 1024,
        ),
    )(A_x, jnp.swapaxes(A_k_cache, 2, 3), jnp.swapaxes(A_v_cache, 2, 3), A_wq, A_wo,
      B_w_r.reshape(1, D), B_w_gate, B_w_up, B_w_down)
```

```python
import functools

import jax
import jax.numpy as jnp
import numpy as np
from jax import lax
import jax.experimental.pallas as pl
import jax.experimental.pallas.tpu as pltpu

S = 2048
D = 640
H = 32
DH = 192
SK = 2048
W = 512
F = 1536
NP = H // 2
TM = 512
NTM = S // TM
LNC = 32
XCH = 512
NXC = S // XCH
OCH = 256
NOC = S // OCH

_NT = (((1,), (1,)), ((), ()))
_F32 = jnp.float32
_BF16 = jnp.bfloat16
_QS = np.float32((DH ** -0.5) * np.log2(np.e))


def _dot(a, b):
    return jnp.dot(a, b, preferred_element_type=_F32)


def _dnt(a, b):
    return lax.dot_general(a, b, _NT, preferred_element_type=_F32)


def _rb(a):
    return a.astype(_BF16).astype(_F32)


def _silu(t):
    h = 0.5 * t
    return h + h * jnp.tanh(h)


def _kernel(x_hbm, k_hbm, v_hbm, wq_hbm, wo_hbm, wr_ref, wg_hbm, wu_hbm, wd_hbm,
            o_hbm,
            x_ref, xn_ref, acc_ref, kp_ref, v_ref, wq_ref, wo_ref, wt_ref,
            wg_ref, wu_ref, wd_ref, o_ref, psem, xsem, fsem, osem):
    p = pl.program_id(0)
    slot = p % 2

    def pair_copies(q, sl):
        c0 = pl.multiple_of(q * (2 * DH), 2 * DH)
        return [
            pltpu.make_async_copy(wq_hbm.at[:, pl.ds(c0, 2 * DH)], wq_ref.at[sl], psem.at[sl, 0]),
            pltpu.make_async_copy(k_hbm.at[0, 2 * q, :, pl.ds(SK - W, W)],
                                  kp_ref.at[sl, 0, pl.ds(0, DH), :], psem.at[sl, 1]),
            pltpu.make_async_copy(k_hbm.at[0, 2 * q + 1, :, pl.ds(SK - W, W)],
                                  kp_ref.at[sl, 1, pl.ds(256 - DH, DH), :], psem.at[sl, 2]),
            pltpu.make_async_copy(v_hbm.at[0, pl.ds(2 * q, 2), :, pl.ds(SK - W, W)],
                                  v_ref.at[sl], psem.at[sl, 3]),
            pltpu.make_async_copy(wo_hbm.at[pl.ds(c0, 2 * DH), :], wo_ref.at[sl], psem.at[sl, 4]),
        ]

    def x_copy(c):
        return pltpu.make_async_copy(x_hbm.at[0, pl.ds(c * XCH, XCH), :],
                                     x_ref.at[pl.ds(c * XCH, XCH), :], xsem.at[c])

    def o_copy(c):
        rows = pl.ds(pl.multiple_of(c * OCH, OCH), OCH)
        return pltpu.make_async_copy(o_ref.at[rows, :], o_hbm.at[0, rows, :], osem.at[c])

    ffn_copies = [
        pltpu.make_async_copy(wg_hbm, wg_ref, fsem.at[0]),
        pltpu.make_async_copy(wu_hbm, wu_ref, fsem.at[1]),
        pltpu.make_async_copy(wd_hbm, wd_ref, fsem.at[2]),
    ]

    def layernorm(r0):
        x = x_ref[r0:r0 + LNC, :].astype(_F32)
        m = jnp.mean(x, axis=-1, keepdims=True)
        d = x - m
        var = jnp.mean(d * d, axis=-1, keepdims=True)
        inv = lax.rsqrt(var + 1e-5)
        xn_ref[r0:r0 + LNC, :] = (d * inv).astype(_BF16)

    def stage_q(r0):
        q2 = _dot(xn_ref[r0:r0 + TM, :], wq_ref[slot])
        return (q2 * _QS).astype(_BF16)

    def stage_s(q2):
        return _dot(q2[:, 0:256], kp_ref[slot, 0]), _dot(q2[:, 128:384], kp_ref[slot, 1])

    def softmax(s):
        e = jnp.exp2(s - jnp.max(s, axis=-1, keepdims=True))
        return (e * (1.0 / jnp.sum(e, axis=-1, keepdims=True))).astype(_BF16)

    def stage_p(s0, s1):
        a = _dnt(v_ref[slot, 0], softmax(s0))
        b = _dnt(v_ref[slot, 1], softmax(s1))
        return jnp.concatenate([a, b], axis=0).astype(_BF16)

    def stage_o(o2t):
        return _dot(wt_ref[...], o2t)

    def attention():
        rs = [u * TM for u in range(NTM)]
        qs = [stage_q(r0) for r0 in rs]
        ss = [stage_s(q) for q in qs]
        os_ = [stage_p(*s) for s in ss]
        return [stage_o(o) for o in os_]

    def router_ffn():
        wr = jnp.broadcast_to(wr_ref[...], (16, D))
        r = _rb(_dnt(wr, xn_ref[...]))[0:8]
        idx = lax.broadcasted_iota(jnp.int32, (8, S), 1)
        m0 = jnp.max(r)
        i0 = jnp.min(jnp.where(r == m0, idx, S))
        r2 = jnp.where(idx == i0, -jnp.inf, r)
        m1 = jnp.max(r2)
        i1 = jnp.min(jnp.where(r2 == m1, idx, S))
        i0 = jnp.minimum(i0, S - 1)
        i1 = jnp.minimum(i1, S - 1)
        row16 = lax.broadcasted_iota(jnp.int32, (16, D), 0)

        def gather(i):
            base = pl.multiple_of((i // 16) * 16, 16)
            blk = xn_ref[pl.ds(base, 16), :].astype(_F32)
            return jnp.sum(jnp.where(row16 == i - base, blk, 0.0), axis=0, keepdims=True)

        x0 = gather(i0)
        x1 = gather(i1)
        xs = jnp.where(row16 == 0, x0, jnp.where(row16 == 1, x1, 0.0)).astype(_BF16)
        gg = _rb(_dot(xs, wg_ref[...]))
        uu = _rb(_dot(xs, wu_ref[...]))
        gg = _rb(_silu(gg))
        y = _rb(_dot((gg * uu).astype(_BF16), wd_ref[...]))
        rs0 = _rb(jax.nn.sigmoid(jnp.full((1, 1), m0, _F32)))
        rs1 = _rb(jax.nn.sigmoid(jnp.full((1, 1), m1, _F32)))
        y0 = _rb(y[0:1] * rs0)
        y1 = _rb(y[1:2] * rs1)

        def scatter_add(i, yrow):
            base = pl.multiple_of((i // 16) * 16, 16)
            blk = xn_ref[pl.ds(base, 16), :].astype(_F32)
            blk = jnp.where(row16 == i - base, blk + yrow, blk)
            xn_ref[pl.ds(base, 16), :] = blk.astype(_BF16)

        scatter_add(i0, y0)
        scatter_add(i1, y1)

    def finish(r0):
        rs = pl.ds(r0, 128)
        for c0 in range(0, D, 128):
            cs = slice(c0, c0 + 128)
            s = acc_ref[cs, rs].T
            t = xn_ref[rs, cs].astype(_F32)
            out = x_ref[rs, cs].astype(_F32) + s * _silu(t)
            o_ref[rs, cs] = out.astype(o_ref.dtype)

    @pl.when(p == 0)
    def _():
        z = jnp.zeros((256 - DH, W), _BF16)
        for sl in range(2):
            kp_ref[sl, 0, DH:256, :] = z
            kp_ref[sl, 1, 0:256 - DH, :] = z
        first = pair_copies(0, 0)
        x_copy(0).start()
        x_copy(1).start()
        acc_ref[...] = jnp.zeros_like(acc_ref)
        later = [[x_copy(2), first[0]], [x_copy(3), first[1], first[2]], [first[3], first[4]], []]
        for c in range(NXC):
            x_copy(c).wait()
            for cp in later[c]:
                cp.start()
            for r0 in range(c * XCH, (c + 1) * XCH, LNC):
                layernorm(r0)
        for c in ffn_copies:
            c.start()

    @pl.when(p + 1 < NP)
    def _():
        for c in pair_copies(p + 1, 1 - slot):
            c.start()

    for c in pair_copies(p, slot):
        c.wait()

    wt_ref[...] = wo_ref[slot].T
    outs = attention()
    for u in range(NTM):
        acc_ref[:, u * TM:(u + 1) * TM] += outs[u]

    @pl.when(p == NP - 1)
    def _():
        for c in ffn_copies:
            c.wait()
        router_ffn()

    @pl.when(p == NP - 1)
    def _():

        @pl.loop(0, NOC)
        def _(c):
            for j in range(OCH // 128):
                finish(pl.multiple_of(c * OCH + j * 128, 128))
            o_copy(c).start()

        for c in range(NOC):
            o_copy(c).wait()


@jax.jit
def pallas_recurrent_scan__sliding_block_cached__moe_arch_mod__prompt_kernel(
    A_x: jax.Array,
    A_k_cache: jax.Array,
    A_v_cache: jax.Array,
    A_wq: jax.Array,
    A_wo: jax.Array,
    B_x: jax.Array,
    B_w_r: jax.Array,
    B_w_gate: jax.Array,
    B_w_up: jax.Array,
    B_w_down: jax.Array,
):
    del B_x
    hbm = pl.BlockSpec(memory_space=pl.ANY)
    return pl.pallas_call(
        _kernel,
        grid=(NP,),
        in_specs=[hbm, hbm, hbm, hbm, hbm,
                  pl.BlockSpec((1, D), lambda p: (0, 0)),
                  hbm, hbm, hbm],
        out_specs=hbm,
        out_shape=jax.ShapeDtypeStruct((1, S, D), A_x.dtype),
        scratch_shapes=[
            pltpu.VMEM((S, D), _BF16),
            pltpu.VMEM((S, D), _BF16),
            pltpu.VMEM((D, S), _F32),
            pltpu.VMEM((2, 2, 256, W), _BF16),
            pltpu.VMEM((2, 2, DH, W), _BF16),
            pltpu.VMEM((2, D, 2 * DH), _BF16),
            pltpu.VMEM((2, 2 * DH, D), _BF16),
            pltpu.VMEM((D, 2 * DH), _BF16),
            pltpu.VMEM((D, F), _BF16),
            pltpu.VMEM((D, F), _BF16),
            pltpu.VMEM((F, D), _BF16),
            pltpu.VMEM((S, D), _BF16),
            pltpu.SemaphoreType.DMA((2, 5)),
            pltpu.SemaphoreType.DMA((NXC,)),
            pltpu.SemaphoreType.DMA((3,)),
            pltpu.SemaphoreType.DMA((NOC,)),
        ],
        compiler_params=pltpu.CompilerParams(
            dimension_semantics=("arbitrary",),
            vmem_limit_bytes=100 * 1024 * 1024,
        ),
    )(A_x, jnp.swapaxes(A_k_cache, 2, 3), jnp.swapaxes(A_v_cache, 2, 3), A_wq, A_wo,
      B_w_r.reshape(1, D), B_w_gate, B_w_up, B_w_down)
```

```python
import functools

import jax
import jax.numpy as jnp
import numpy as np
from jax import lax
import jax.experimental.pallas as pl
import jax.experimental.pallas.tpu as pltpu

S = 2048
D = 640
H = 32
DH = 192
SK = 2048
W = 512
F = 1536
NP = H // 2
TM = 512
NTM = S // TM
LNC = 32
XCH = 512
NXC = S // XCH
OCH = 256
NOC = S // OCH

_NT = (((1,), (1,)), ((), ()))
_F32 = jnp.float32
_BF16 = jnp.bfloat16
_QS = np.float32((DH ** -0.5) * np.log2(np.e))


def _dot(a, b):
    return jnp.dot(a, b, preferred_element_type=_F32)


def _dnt(a, b):
    return lax.dot_general(a, b, _NT, preferred_element_type=_F32)


def _rb(a):
    return a.astype(_BF16).astype(_F32)


def _silu(t):
    h = 0.5 * t
    return h + h * jnp.tanh(h)


def _kernel(x_hbm, k_hbm, v_hbm, wq_hbm, wo_hbm, wr_ref, wg_hbm, wu_hbm, wd_hbm,
            o_hbm,
            x_ref, xn_ref, acc_ref, kp_ref, v_ref, wq_ref, wo_ref, wt_ref,
            wg_ref, wu_ref, wd_ref, o_ref, r_ref, psem, xsem, fsem, osem):
    p = pl.program_id(0)
    slot = p % 2

    def pair_copies(q, sl):
        c0 = pl.multiple_of(q * (2 * DH), 2 * DH)
        return [
            pltpu.make_async_copy(wq_hbm.at[:, pl.ds(c0, 2 * DH)], wq_ref.at[sl], psem.at[sl, 0]),
            pltpu.make_async_copy(k_hbm.at[0, 2 * q, :, pl.ds(SK - W, W)],
                                  kp_ref.at[sl, 0, pl.ds(0, DH), :], psem.at[sl, 1]),
            pltpu.make_async_copy(k_hbm.at[0, 2 * q + 1, :, pl.ds(SK - W, W)],
                                  kp_ref.at[sl, 1, pl.ds(256 - DH, DH), :], psem.at[sl, 2]),
            pltpu.make_async_copy(v_hbm.at[0, pl.ds(2 * q, 2), :, pl.ds(SK - W, W)],
                                  v_ref.at[sl], psem.at[sl, 3]),
            pltpu.make_async_copy(wo_hbm.at[pl.ds(c0, 2 * DH), :], wo_ref.at[sl], psem.at[sl, 4]),
        ]

    def x_copy(c):
        return pltpu.make_async_copy(x_hbm.at[0, pl.ds(c * XCH, XCH), :],
                                     x_ref.at[pl.ds(c * XCH, XCH), :], xsem.at[c])

    def o_copy(c):
        rows = pl.ds(pl.multiple_of(c * OCH, OCH), OCH)
        return pltpu.make_async_copy(o_ref.at[rows, :], o_hbm.at[0, rows, :], osem.at[c])

    ffn_copies = [
        pltpu.make_async_copy(wg_hbm, wg_ref, fsem.at[0]),
        pltpu.make_async_copy(wu_hbm, wu_ref, fsem.at[1]),
        pltpu.make_async_copy(wd_hbm, wd_ref, fsem.at[2]),
    ]

    def layernorm(r0):
        x = x_ref[r0:r0 + LNC, :].astype(_F32)
        m = jnp.mean(x, axis=-1, keepdims=True)
        d = x - m
        var = jnp.mean(d * d, axis=-1, keepdims=True)
        inv = lax.rsqrt(var + 1e-5)
        xn_ref[r0:r0 + LNC, :] = (d * inv).astype(_BF16)

    def stage_q(r0):
        q2 = _dot(xn_ref[r0:r0 + TM, :], wq_ref[slot])
        return (q2 * _QS).astype(_BF16)

    def stage_s(q2):
        return _dot(q2[:, 0:256], kp_ref[slot, 0]), _dot(q2[:, 128:384], kp_ref[slot, 1])

    def softmax(s):
        e = jnp.exp2(s - jnp.max(s, axis=-1, keepdims=True))
        return (e * (1.0 / jnp.sum(e, axis=-1, keepdims=True))).astype(_BF16)

    def stage_p(s0, s1):
        a = _dnt(v_ref[slot, 0], softmax(s0))
        b = _dnt(v_ref[slot, 1], softmax(s1))
        return jnp.concatenate([a, b], axis=0).astype(_BF16)

    def stage_o(o2t):
        return _dot(wt_ref[...], o2t)

    def attention():
        rs = [u * TM for u in range(NTM)]
        qs = [stage_q(r0) for r0 in rs]
        ss = [stage_s(q) for q in qs]
        os_ = [stage_p(*s) for s in ss]
        return [stage_o(o) for o in os_]

    def router_ffn():
        r = r_ref[...]
        idx = lax.broadcasted_iota(jnp.int32, (8, S), 1)
        m0 = jnp.max(r)
        i0 = jnp.min(jnp.where(r == m0, idx, S))
        r2 = jnp.where(idx == i0, -jnp.inf, r)
        m1 = jnp.max(r2)
        i1 = jnp.min(jnp.where(r2 == m1, idx, S))
        i0 = jnp.minimum(i0, S - 1)
        i1 = jnp.minimum(i1, S - 1)
        row16 = lax.broadcasted_iota(jnp.int32, (16, D), 0)

        def gather(i):
            base = pl.multiple_of((i // 16) * 16, 16)
            blk = xn_ref[pl.ds(base, 16), :].astype(_F32)
            return jnp.sum(jnp.where(row16 == i - base, blk, 0.0), axis=0, keepdims=True)

        x0 = gather(i0)
        x1 = gather(i1)
        xs = jnp.where(row16 == 0, x0, jnp.where(row16 == 1, x1, 0.0)).astype(_BF16)
        gg = _rb(_dot(xs, wg_ref[...]))
        uu = _rb(_dot(xs, wu_ref[...]))
        gg = _rb(_silu(gg))
        y = _rb(_dot((gg * uu).astype(_BF16), wd_ref[...]))
        rs0 = _rb(jax.nn.sigmoid(jnp.full((1, 1), m0, _F32)))
        rs1 = _rb(jax.nn.sigmoid(jnp.full((1, 1), m1, _F32)))
        y0 = _rb(y[0:1] * rs0)
        y1 = _rb(y[1:2] * rs1)

        def scatter_add(i, yrow):
            base = pl.multiple_of((i // 16) * 16, 16)
            blk = xn_ref[pl.ds(base, 16), :].astype(_F32)
            blk = jnp.where(row16 == i - base, blk + yrow, blk)
            xn_ref[pl.ds(base, 16), :] = blk.astype(_BF16)

        scatter_add(i0, y0)
        scatter_add(i1, y1)

    def finish(r0):
        rs = pl.ds(r0, 128)
        for c0 in range(0, D, 128):
            cs = slice(c0, c0 + 128)
            s = acc_ref[cs, rs].T
            t = xn_ref[rs, cs].astype(_F32)
            out = x_ref[rs, cs].astype(_F32) + s * _silu(t)
            o_ref[rs, cs] = out.astype(o_ref.dtype)

    @pl.when(p == 0)
    def _():
        z = jnp.zeros((256 - DH, W), _BF16)
        for sl in range(2):
            kp_ref[sl, 0, DH:256, :] = z
            kp_ref[sl, 1, 0:256 - DH, :] = z
        first = pair_copies(0, 0)
        x_copy(0).start()
        x_copy(1).start()
        acc_ref[...] = jnp.zeros_like(acc_ref)
        later = [[x_copy(2), first[0]], [x_copy(3), first[1], first[2]], [first[3], first[4]], []]
        for c in range(NXC):
            x_copy(c).wait()
            for cp in later[c]:
                cp.start()
            for r0 in range(c * XCH, (c + 1) * XCH, LNC):
                layernorm(r0)
            wr = jnp.broadcast_to(wr_ref[...].reshape(1, D), (16, D))
            rc = _dnt(wr, xn_ref[c * XCH:(c + 1) * XCH, :])
            r_ref[:, c * XCH:(c + 1) * XCH] = _rb(rc[0:8])
        for c in ffn_copies:
            c.start()

    @pl.when(p + 1 < NP)
    def _():
        for c in pair_copies(p + 1, 1 - slot):
            c.start()

    for c in pair_copies(p, slot):
        c.wait()

    @pl.when(p < NP - 1)
    def _():
        wt_ref[...] = wo_ref[slot].T
        outs = attention()
        for u in range(NTM):
            acc_ref[:, u * TM:(u + 1) * TM] += outs[u]

    @pl.when(p == NP - 1)
    def _():
        for c in ffn_copies:
            c.wait()
        wt_ref[...] = wo_ref[slot].T
        qs = [stage_q(u * TM) for u in range(NTM)]
        router_ffn()
        ss = [stage_s(q) for q in qs]
        os_ = [stage_p(*s) for s in ss]
        for u in range(NTM):
            acc_ref[:, u * TM:(u + 1) * TM] += stage_o(os_[u])
            for j in range(TM // 128):
                finish(u * TM + j * 128)
                if j % 2 == 1:
                    o_copy(u * 2 + j // 2).start()
        for c in range(NOC):
            o_copy(c).wait()


@jax.jit
def pallas_recurrent_scan__sliding_block_cached__moe_arch_mod__prompt_kernel(
    A_x: jax.Array,
    A_k_cache: jax.Array,
    A_v_cache: jax.Array,
    A_wq: jax.Array,
    A_wo: jax.Array,
    B_x: jax.Array,
    B_w_r: jax.Array,
    B_w_gate: jax.Array,
    B_w_up: jax.Array,
    B_w_down: jax.Array,
):
    del B_x
    hbm = pl.BlockSpec(memory_space=pl.ANY)
    return pl.pallas_call(
        _kernel,
        grid=(NP,),
        in_specs=[hbm, hbm, hbm, hbm, hbm,
                  pl.BlockSpec((D,), lambda p: (0,)),
                  hbm, hbm, hbm],
        out_specs=hbm,
        out_shape=jax.ShapeDtypeStruct((1, S, D), A_x.dtype),
        scratch_shapes=[
            pltpu.VMEM((S, D), _BF16),
            pltpu.VMEM((S, D), _BF16),
            pltpu.VMEM((D, S), _F32),
            pltpu.VMEM((2, 2, 256, W), _BF16),
            pltpu.VMEM((2, 2, DH, W), _BF16),
            pltpu.VMEM((2, D, 2 * DH), _BF16),
            pltpu.VMEM((2, 2 * DH, D), _BF16),
            pltpu.VMEM((D, 2 * DH), _BF16),
            pltpu.VMEM((D, F), _BF16),
            pltpu.VMEM((D, F), _BF16),
            pltpu.VMEM((F, D), _BF16),
            pltpu.VMEM((S, D), _BF16),
            pltpu.VMEM((8, S), _F32),
            pltpu.SemaphoreType.DMA((2, 5)),
            pltpu.SemaphoreType.DMA((NXC,)),
            pltpu.SemaphoreType.DMA((3,)),
            pltpu.SemaphoreType.DMA((NOC,)),
        ],
        compiler_params=pltpu.CompilerParams(
            dimension_semantics=("arbitrary",),
            vmem_limit_bytes=100 * 1024 * 1024,
        ),
    )(A_x, jnp.swapaxes(A_k_cache, 2, 3), jnp.swapaxes(A_v_cache, 2, 3), A_wq, A_wo,
      B_w_r, B_w_gate, B_w_up, B_w_down)
```

```python
import jax
import jax.numpy as jnp
import numpy as np
from jax import lax
import jax.experimental.pallas as pl
import jax.experimental.pallas.tpu as pltpu

S = 2048
D = 640
H = 32
DH = 192
SK = 2048
W = 512
F = 1536
NP = H // 2
TM = 256
NTM = S // TM
LNC = 32
XCH = 512
NXC = S // XCH
OCH = 256
NOC = S // OCH

_NT = (((1,), (1,)), ((), ()))
_F32 = jnp.float32
_BF16 = jnp.bfloat16
_QS = np.float32((DH ** -0.5) * np.log2(np.e))


def _dot(a, b):
    return jnp.dot(a, b, preferred_element_type=_F32)


def _dnt(a, b):
    return lax.dot_general(a, b, _NT, preferred_element_type=_F32)


def _rb(a):
    return a.astype(_BF16).astype(_F32)


def _silu(t):
    h = 0.5 * t
    return h + h * jnp.tanh(h)


def _kernel(x_hbm, k_hbm, v_hbm, wq_hbm, wo_hbm, wr_hbm, wg_hbm, wu_hbm, wd_hbm,
            o_hbm,
            x_ref, xn_ref, acc_ref, kp_ref, v_ref, wq_ref, wo_ref, wt_ref,
            wg_ref, wu_ref, wd_ref, o_ref, r_ref, wr_ref, psem, xsem, fsem, osem):
    p = pl.program_id(0)
    slot = p % 2

    def pair_copies(q, sl):
        c0 = pl.multiple_of(q * (2 * DH), 2 * DH)
        return [
            pltpu.make_async_copy(wq_hbm.at[:, pl.ds(c0, 2 * DH)], wq_ref.at[sl], psem.at[sl, 0]),
            pltpu.make_async_copy(k_hbm.at[0, 2 * q, :, pl.ds(SK - W, W)],
                                  kp_ref.at[sl, 0, pl.ds(0, DH), :], psem.at[sl, 1]),
            pltpu.make_async_copy(k_hbm.at[0, 2 * q + 1, :, pl.ds(SK - W, W)],
                                  kp_ref.at[sl, 1, pl.ds(256 - DH, DH), :], psem.at[sl, 2]),
            pltpu.make_async_copy(v_hbm.at[0, pl.ds(2 * q, 2), :, pl.ds(SK - W, W)],
                                  v_ref.at[sl], psem.at[sl, 3]),
            pltpu.make_async_copy(wo_hbm.at[pl.ds(c0, 2 * DH), :], wo_ref.at[sl], psem.at[sl, 4]),
        ]

    def x_copy(c):
        return pltpu.make_async_copy(x_hbm.at[0, pl.ds(c * XCH, XCH), :],
                                     x_ref.at[pl.ds(c * XCH, XCH), :], xsem.at[c])

    def o_copy(c):
        rows = pl.ds(pl.multiple_of(c * OCH, OCH), OCH)
        return pltpu.make_async_copy(o_ref.at[rows, :], o_hbm.at[0, rows, :], osem.at[c])

    ffn_copies = [
        pltpu.make_async_copy(wg_hbm, wg_ref, fsem.at[0]),
        pltpu.make_async_copy(wu_hbm, wu_ref, fsem.at[1]),
        pltpu.make_async_copy(wd_hbm, wd_ref, fsem.at[2]),
    ]

    wr_copy = pltpu.make_async_copy(wr_hbm, wr_ref, fsem.at[3])

    def layernorm(r0):
        x = x_ref[r0:r0 + LNC, :].astype(_F32)
        m = jnp.mean(x, axis=-1, keepdims=True)
        d = x - m
        var = jnp.mean(d * d, axis=-1, keepdims=True)
        inv = lax.rsqrt(var + 1e-5)
        xn_ref[r0:r0 + LNC, :] = (d * inv).astype(_BF16)

    def stage_q(r0):
        q2 = _dot(xn_ref[r0:r0 + TM, :], wq_ref[slot])
        return (q2 * _QS).astype(_BF16)

    def stage_s(q2):
        return _dot(q2[:, 0:256], kp_ref[slot, 0]), _dot(q2[:, 128:384], kp_ref[slot, 1])

    def softmax(s):
        e = jnp.exp2(s - jnp.max(s, axis=-1, keepdims=True))
        return (e * (1.0 / jnp.sum(e, axis=-1, keepdims=True))).astype(_BF16)

    def stage_p(s0, s1):
        a = _dnt(v_ref[slot, 0], softmax(s0))
        b = _dnt(v_ref[slot, 1], softmax(s1))
        return jnp.concatenate([a, b], axis=0).astype(_BF16)

    def stage_o(o2t):
        return _dot(wt_ref[...], o2t)

    def attention():
        rs = [u * TM for u in range(NTM)]
        qs = [stage_q(r0) for r0 in rs]
        ss = [stage_s(q) for q in qs]
        os_ = [stage_p(*s) for s in ss]
        return [stage_o(o) for o in os_]

    def router_ffn():
        r = r_ref[...]
        idx = lax.broadcasted_iota(jnp.int32, (8, S), 1)
        m0 = jnp.max(r)
        i0 = jnp.min(jnp.where(r == m0, idx, S))
        r2 = jnp.where(idx == i0, -jnp.inf, r)
        m1 = jnp.max(r2)
        i1 = jnp.min(jnp.where(r2 == m1, idx, S))
        i0 = jnp.clip(i0, 0, S - 1)
        i1 = jnp.clip(i1, 0, S - 1)
        row16 = lax.broadcasted_iota(jnp.int32, (16, D), 0)

        def gather(i):
            base = pl.multiple_of((i // 16) * 16, 16)
            blk = xn_ref[pl.ds(base, 16), :].astype(_F32)
            return jnp.sum(jnp.where(row16 == i - base, blk, 0.0), axis=0, keepdims=True)

        x0 = gather(i0)
        x1 = gather(i1)
        xs = jnp.where(row16 == 0, x0, jnp.where(row16 == 1, x1, 0.0)).astype(_BF16)
        gg = _rb(_dot(xs, wg_ref[...]))
        uu = _rb(_dot(xs, wu_ref[...]))
        gg = _rb(_silu(gg))
        y = _rb(_dot((gg * uu).astype(_BF16), wd_ref[...]))
        rs0 = _rb(jax.nn.sigmoid(jnp.full((1, 1), m0, _F32)))
        rs1 = _rb(jax.nn.sigmoid(jnp.full((1, 1), m1, _F32)))
        y0 = _rb(y[0:1] * rs0)
        y1 = _rb(y[1:2] * rs1)

        def scatter_add(i, yrow):
            base = pl.multiple_of((i // 16) * 16, 16)
            blk = xn_ref[pl.ds(base, 16), :].astype(_F32)
            blk = jnp.where(row16 == i - base, blk + yrow, blk)
            xn_ref[pl.ds(base, 16), :] = blk.astype(_BF16)

        scatter_add(i0, y0)
        scatter_add(i1, y1)

    def finish(r0):
        rs = pl.ds(r0, 128)
        for c0 in range(0, D, 128):
            cs = slice(c0, c0 + 128)
            s = acc_ref[cs, rs].T
            t = xn_ref[rs, cs].astype(_F32)
            out = x_ref[rs, cs].astype(_F32) + s * _silu(t)
            o_ref[rs, cs] = out.astype(o_ref.dtype)

    @pl.when(p == 0)
    def _():
        z = jnp.zeros((256 - DH, W), _BF16)
        for sl in range(2):
            kp_ref[sl, 0, DH:256, :] = z
            kp_ref[sl, 1, 0:256 - DH, :] = z
        first = pair_copies(0, 0)
        x_copy(0).start()
        wr_copy.start()
        x_copy(1).start()
        acc_ref[...] = jnp.zeros_like(acc_ref)
        later = [[x_copy(2), first[0]], [x_copy(3), first[1], first[2]], [first[3], first[4]], []]
        for c in range(NXC):
            x_copy(c).wait()
            if c == 0:
                wr_copy.wait()
            for cp in later[c]:
                cp.start()
            for r0 in range(c * XCH, (c + 1) * XCH, LNC):
                layernorm(r0)
            wr = jnp.broadcast_to(wr_ref[...].reshape(1, D), (16, D))
            rc = _dnt(wr, xn_ref[c * XCH:(c + 1) * XCH, :])
            r_ref[:, c * XCH:(c + 1) * XCH] = _rb(rc[0:8])
        for c in ffn_copies:
            c.start()

    @pl.when(p < NP - 1)
    def _():
        for c in pair_copies(p, slot):
            c.wait()
        for c in pair_copies(p + 1, 1 - slot):
            c.start()
        wt_ref[...] = wo_ref[slot].T
        outs = attention()
        for u in range(NTM):
            acc_ref[:, u * TM:(u + 1) * TM] += outs[u]

    @pl.when(p == NP - 1)
    def _():
        for c in pair_copies(p, slot):
            c.wait()
        for c in ffn_copies:
            c.wait()
        wt_ref[...] = wo_ref[slot].T
        qs = [stage_q(u * TM) for u in range(NTM)]
        router_ffn()
        ss = [stage_s(q) for q in qs]
        os_ = [stage_p(*s) for s in ss]
        for u in range(NTM):
            acc_ref[:, u * TM:(u + 1) * TM] += stage_o(os_[u])
            for j in range(TM // 128):
                finish(u * TM + j * 128)
                row_end = u * TM + (j + 1) * 128
                if row_end % OCH == 0:
                    o_copy(row_end // OCH - 1).start()
        for c in range(NOC):
            o_copy(c).wait()


@jax.jit
def pallas_recurrent_scan__sliding_block_cached__moe_arch_mod__prompt_kernel(
    A_x: jax.Array,
    A_k_cache: jax.Array,
    A_v_cache: jax.Array,
    A_wq: jax.Array,
    A_wo: jax.Array,
    B_x: jax.Array,
    B_w_r: jax.Array,
    B_w_gate: jax.Array,
    B_w_up: jax.Array,
    B_w_down: jax.Array,
):
    del B_x
    hbm = pl.BlockSpec(memory_space=pl.ANY)
    return pl.pallas_call(
        _kernel,
        grid=(NP,),
        in_specs=[hbm, hbm, hbm, hbm, hbm,
                  hbm,
                  hbm, hbm, hbm],
        out_specs=hbm,
        out_shape=jax.ShapeDtypeStruct((1, S, D), A_x.dtype),
        scratch_shapes=[
            pltpu.VMEM((S, D), _BF16),
            pltpu.VMEM((S, D), _BF16),
            pltpu.VMEM((D, S), _F32),
            pltpu.VMEM((2, 2, 256, W), _BF16),
            pltpu.VMEM((2, 2, DH, W), _BF16),
            pltpu.VMEM((2, D, 2 * DH), _BF16),
            pltpu.VMEM((2, 2 * DH, D), _BF16),
            pltpu.VMEM((D, 2 * DH), _BF16),
            pltpu.VMEM((D, F), _BF16),
            pltpu.VMEM((D, F), _BF16),
            pltpu.VMEM((F, D), _BF16),
            pltpu.VMEM((S, D), _BF16),
            pltpu.VMEM((8, S), _F32),
            pltpu.VMEM((D,), _BF16),
            pltpu.SemaphoreType.DMA((2, 5)),
            pltpu.SemaphoreType.DMA((NXC,)),
            pltpu.SemaphoreType.DMA((4,)),
            pltpu.SemaphoreType.DMA((NOC,)),
        ],
        compiler_params=pltpu.CompilerParams(
            dimension_semantics=("arbitrary",),
            vmem_limit_bytes=100 * 1024 * 1024,
        ),
    )(A_x, jnp.swapaxes(A_k_cache, 2, 3), jnp.swapaxes(A_v_cache, 2, 3), A_wq, A_wo,
      B_w_r, B_w_gate, B_w_up, B_w_down)
```
